```python
import jax
import jax.numpy as jnp

def _softmax(x, axis=-1):
    return jax.nn.softmax(x, axis=axis)
def _gelu(x):
    return jax.nn.gelu(x, approximate=True)
def _silu(x):
    return jax.nn.silu(x)
def _sigmoid(x):
    return jax.nn.sigmoid(x)
def _layernorm(x, axis=-1, eps=1e-5):
    m = jnp.mean(x, axis=axis, keepdims=True)
    v = jnp.var(x, axis=axis, keepdims=True)
    return (x - m) / jnp.sqrt(v + eps)
def _scatter_add(tgt, idx, src, axis=0):
    return tgt.at[idx].add(src)
def _segment_sum(src, seg, n):
    return jax.ops.segment_sum(src, seg, n)
class _Rng:
    def __init__(self, key):
        self._k = key
    def _next(self):
        self._k, sub = jax.random.split(self._k)
        return sub
    def normal(self, shape):
        return jax.random.normal(self._next(), shape, dtype=jnp.bfloat16)
    def randint(self, lo, hi, shape):
        return jax.random.randint(self._next(), shape, lo, hi, dtype=jnp.int32)
    def uniform(self, shape, lo=0.0, hi=1.0):
        return jax.random.uniform(self._next(), shape, jnp.bfloat16, lo, hi)
    def permutation(self, n):
        return jax.random.permutation(self._next(), n)


kernel_name = 'concat_heads__ssm_conv_h3__linear_attn_block__prompt'

def setup_inputs():
    _rng = _Rng(jax.random.key(int.from_bytes(__import__("os").urandom(4), "little")))
    _w = (lambda a: (lambda t: t.astype(jnp.bfloat16) if jnp.issubdtype(t.dtype, jnp.floating) else t)(jnp.asarray(a)))
    def _A_setup():
        B, S, D = 1, 2048, 1024
        ks = 4
        return {
            "q": _w((lambda *s: _rng.normal(s) * 0.05)(B, S, D)),
            "k": _w((lambda *s: _rng.normal(s) * 0.05)(B, S, D)),
            "v": _w((lambda *s: _rng.normal(s) * 0.05)(B, S, D)),
            "shift_k": _w((lambda *s: _rng.normal(s) * 0.05)(D, ks) * 0.5),
            "ssm_k": _w((lambda *s: _rng.normal(s) * 0.05)(D, S) * (1.0 / S ** 0.5)),
            "ssm_D": _w((lambda *s: _rng.normal(s) * 0.05)(D)),
        }
    _A_in = _A_setup()

    def _B_setup():
        B, S, D = 1, 2048, 1024
        return {
            "x": _w((lambda *s: _rng.normal(s) * 0.05)(B, S, D)),
            "wqkv": _w((lambda *s: _rng.normal(s) * 0.05)(D, 3 * D)),
            "wo": _w((lambda *s: _rng.normal(s) * 0.05)(D, D)),
        }
    _B_in = _B_setup()

    return {
        "A_q": _A_in["q"],
        "A_k": _A_in["k"],
        "A_v": _A_in["v"],
        "A_shift_k": _A_in["shift_k"],
        "A_ssm_k": _A_in["ssm_k"],
        "A_ssm_D": _A_in["ssm_D"],
        "B_x": _B_in["x"],
        "B_wqkv": _B_in["wqkv"],
        "B_wo": _B_in["wo"],
    }

def reference(A_q, A_k, A_v, A_shift_k, A_ssm_k, A_ssm_D, B_x, B_wqkv, B_wo):
    def _A_ref(q, k, v, shift_k, ssm_k, ssm_D):
        B, S, D = q.shape
        ks = shift_k.shape[-1]
        k_pad = jnp.pad(k, ((0, 0), (ks - 1, 0), (0, 0)))
        k_shift = jnp.zeros_like(k)
        for t in range(ks):
            k_shift = k_shift + k_pad[:, t:t + S, :] * shift_k[:, ks - 1 - t][None, None, :]
        kv = k_shift * v
        L = 2 * S
        kv_pad = jnp.pad(kv, ((0, 0), (0, S), (0, 0)))
        kf_pad = jnp.pad(ssm_k, ((0, 0), (0, S)))
        kv_f = (lambda x, axes=(-2,-1): jnp.fft.rfft2(x.astype(jnp.float32), axes=axes))(kv_pad[:, None, :, :], axes=(1, 2))
        kf_f = (lambda x, axes=(-2,-1): jnp.fft.rfft2(x.astype(jnp.float32), axes=axes))(kf_pad[:, None, :], axes=(1, 2))
        kf_f = (lambda x, *d: x.transpose(*d))(kf_f, 1, 2, 0)
        y_f = kv_f * kf_f[None, :, :, :]
        y = (lambda x, s, axes=(-2,-1): jnp.fft.irfft2(x, s=s, axes=axes).astype(jnp.bfloat16))(y_f, (1, L), axes=(1, 2))[:, 0, :S, :]
        y = y + kv * ssm_D[None, None, :]
        return q * y

    def _B_ref(x, wqkv, wo):
        B, S, D = x.shape
        H = 32; Dh = D // H
        qkv = (lambda x, *d: x.transpose(*d))((x @ wqkv).reshape(B, S, 3, H, Dh), 2, 0, 3, 1, 4)
        q, k, v = qkv[0], qkv[1], qkv[2]
        phi = lambda t: jnp.where(t > 0, t + 1, jnp.exp(t)) + 1e-6
        pq, pk = phi(q), phi(k)
        kv = jnp.einsum("bhsd,bhse->bhde", pk, v)
        z = jnp.einsum("bhsd->bhd", pk)
        num = jnp.einsum("bhqd,bhde->bhqe", pq, kv)
        den = jnp.einsum("bhqd,bhd->bhq", pq, z)[..., None] + 1e-6
        o = num / den
        return (lambda x, *d: x.transpose(*d))(o, 0, 2, 1, 3).reshape(B, S, D) @ wo

    a = _A_ref(A_q, A_k, A_v, A_shift_k, A_ssm_k, A_ssm_D)
    b = _B_ref(B_x, B_wqkv, B_wo)
    return jnp.concatenate([a, b], axis=-1)
```

```python
import numpy as np
import jax
import jax.numpy as jnp
from jax import lax
import jax.experimental.pallas as pl
import jax.experimental.pallas.tpu as pltpu

S = 2048
D = 1024
CT = 128
NG = D // CT
L = 128
NC = S // L
TB = 256
NJ = S // TB
PAD = 16
DH = 32

F32 = jnp.float32
BF16 = jnp.bfloat16


def _dft_mats():
    f = np.concatenate([np.arange(0, L, 2), np.arange(1, L, 2)]).astype(np.float64)
    a = np.arange(L, dtype=np.float64)
    ang = 2.0 * np.pi * np.outer(f + 0.5, a) / (2 * L)
    fwd = np.concatenate([np.cos(ang), -np.sin(ang)], axis=0)
    inv = fwd.T / L
    return fwd.astype(BF16), inv.astype(BF16)


def _phi(t):
    return jnp.where(t > 0, t + 1.0, jnp.exp(t)) + 1e-6


def _kernel(q_hbm, k_hbm, v_hbm, shk_ref, ssm_hbm, d_ref, x_hbm, w_hbm, wo_hbm,
            f_ref, g_ref, out_hbm,
            qb, kb, vb, sb, xb, wb, wob, u_s, kf_s, y_s, pk_s, pqn_s, m_s,
            par_s, oa_s, ob_s, in_sem, x_sem, oa_sem, ob_sem):

    def in_copies(g):
        c = pl.multiple_of(g * CT, CT)
        return [
            pltpu.make_async_copy(w_hbm.at[:, pl.ds(D + c, CT)], wb.at[g, :, pl.ds(0, CT)], in_sem.at[0, g]),
            pltpu.make_async_copy(k_hbm.at[:, pl.ds(c, CT)], kb.at[g, pl.ds(PAD, S), :], in_sem.at[1, g]),
            pltpu.make_async_copy(v_hbm.at[:, pl.ds(c, CT)], vb.at[g], in_sem.at[2, g]),
            pltpu.make_async_copy(ssm_hbm.at[pl.ds(c, CT), :], sb.at[g], in_sem.at[3, g]),
            pltpu.make_async_copy(w_hbm.at[:, pl.ds(2 * D + c, CT)], wb.at[g, :, pl.ds(CT, CT)], in_sem.at[4, g]),
            pltpu.make_async_copy(w_hbm.at[:, pl.ds(c, CT)], wb.at[g, :, pl.ds(2 * CT, CT)], in_sem.at[5, g]),
            pltpu.make_async_copy(wo_hbm.at[pl.ds(c, CT), :], wob.at[g], in_sem.at[6, g]),
            pltpu.make_async_copy(q_hbm.at[:, pl.ds(c, CT)], qb.at[g], in_sem.at[7, g]),
        ]

    def x_copy(j):
        r = pl.multiple_of(j * TB, TB)
        return pltpu.make_async_copy(x_hbm.at[pl.ds(r, TB), :], xb.at[pl.ds(r, TB), :], x_sem.at[j])

    def oa_copy(g):
        c = pl.multiple_of(g * CT, CT)
        return pltpu.make_async_copy(oa_s.at[g], out_hbm.at[:, pl.ds(c, CT)], oa_sem.at[g])

    def ob_copy(j):
        r = pl.multiple_of(j * TB, TB)
        return pltpu.make_async_copy(ob_s.at[j], out_hbm.at[pl.ds(r, TB), pl.ds(D, D)], ob_sem.at[j])

    c0 = in_copies(0)
    c0[0].start()
    x_copy(0).start()
    for cp in c0[1:4]:
        cp.start()
    for j in range(1, NJ):
        x_copy(j).start()
    for cp in c0[4:]:
        cp.start()

    for g in range(NG):
        kb[g, 0:PAD, :] = jnp.zeros((PAD, CT), BF16)
    par_s[0:4, :] = shk_ref[...].astype(F32).T
    par_s[4:5, :] = d_ref[...].astype(F32)

    ri = lax.broadcasted_iota(jnp.int32, (CT, CT), 0) // DH
    ci = lax.broadcasted_iota(jnp.int32, (CT, CT), 1) // DH
    bd_mask = ri == ci

    def g_body(g, carry):
        cps = in_copies(g)

        @pl.when(g + 1 < NG)
        def _():
            for cp in in_copies(g + 1):
                cp.start()

        for cp in cps[0:4]:
            cp.wait()
        c = pl.multiple_of(g * CT, CT)
        par = par_s[:, pl.ds(c, CT)]

        def loop1(j, z):
            @pl.when(g == 0)
            def _():
                x_copy(j).wait()
            r = pl.multiple_of(j * TB, TB)
            kk = jnp.dot(xb[pl.ds(r, TB), :], wb[g, :, 0:CT], preferred_element_type=F32)
            pk = _phi(kk)
            pk_s[pl.ds(r, TB), :] = pk.astype(BF16)
            z = z + pk.reshape(TB // 8, 8, CT).sum(axis=0)
            ka = kb[g, pl.ds(r, TB + PAD), :].astype(F32)
            ks = ka[PAD:PAD + TB] * par[0:1]
            for t in range(1, 4):
                ks = ks + ka[PAD - t:PAD - t + TB] * par[t:t + 1]
            kv = (ks * vb[g, pl.ds(r, TB), :].astype(F32)).astype(BF16)
            fm = f_ref[...]
            for h in range(TB // L):
                ch = j * (TB // L) + h
                u_s[ch] = jnp.dot(fm, kv[h * L:(h + 1) * L], preferred_element_type=F32)
                kt = sb[g, :, pl.ds(pl.multiple_of(r + h * L, L), L)]
                kf_s[ch] = lax.dot_general(fm, kt, (((1,), (1,)), ((), ())),
                                           preferred_element_type=F32)
            return z

        z = lax.fori_loop(0, NJ, loop1, jnp.zeros((8, CT), F32))
        z = jnp.sum(z, axis=0, keepdims=True)
        zbd_t = jnp.where(bd_mask, z, 0.0).astype(BF16)
        cps[4].wait()
        cps[5].wait()
        dvec = par[4:5]

        def loop2(j, kvacc):
            r = pl.multiple_of(j * TB, TB)
            vq = jnp.dot(xb[pl.ds(r, TB), :], wb[g, :, CT:3 * CT], preferred_element_type=F32)
            vv = vq[:, 0:CT].astype(BF16)
            kvacc = kvacc + lax.dot_general(pk_s[pl.ds(r, TB), :], vv, (((0,), (0,)), ((), ())),
                                            preferred_element_type=F32)
            pq = _phi(vq[:, CT:2 * CT])
            den = lax.dot_general(pq.astype(BF16), zbd_t, (((1,), (1,)), ((), ())),
                                  preferred_element_type=F32) + 1e-6
            pqn_s[g, pl.ds(r, TB), :] = (pq / den).astype(BF16)
            rows = L // NJ
            p = pl.multiple_of(j * rows, rows)
            sgn = jnp.where(j < NJ // 2, 1.0, -1.0).astype(F32)

            def ld(ref, ch):
                return ref[ch, pl.ds(p, rows), :], ref[ch, pl.ds(L + p, rows), :]

            prev = None
            B = 4
            for cb in range(NC // B):
                acc = [None] * B
                for jb in range(cb + 1):
                    us = [ld(u_s, jb * B + i) for i in range(B)]
                    for m in range((cb - jb) * B - (B - 1), (cb - jb) * B + B):
                        if m < 0:
                            continue
                        kr, ki = ld(kf_s, m)
                        if m == 0:
                            kr = kr + dvec
                        for i in range(B):
                            cc = jb * B + i + m - cb * B
                            if 0 <= cc < B:
                                ur, ui = us[i]
                                tr = ur * kr - ui * ki
                                ti = ur * ki + ui * kr
                                if acc[cc] is None:
                                    acc[cc] = (tr, ti)
                                else:
                                    acc[cc] = (acc[cc][0] + tr, acc[cc][1] + ti)
                for i in range(B):
                    yr, yi = acc[i]
                    if prev is not None:
                        yr, yi = yr - sgn * prev[1], yi + sgn * prev[0]
                    prev = acc[i]
                    y_s[cb * B + i, pl.ds(p, rows), :] = yr.astype(BF16)
                    y_s[cb * B + i, pl.ds(L + p, rows), :] = yi.astype(BF16)
            return kvacc

        kvacc = lax.fori_loop(0, NJ, loop2, jnp.zeros((CT, CT), F32))
        cps[6].wait()
        cps[7].wait()
        kvm = jnp.where(bd_mask, kvacc, 0.0).astype(BF16)
        m_s[pl.ds(c, CT), :] = jnp.dot(kvm, wob[g], preferred_element_type=F32).astype(BF16)

        def loop3(j, carry):
            gm = g_ref[...]
            for h in range(TB // L):
                ch = j * (TB // L) + h
                rr = pl.multiple_of(ch * L, L)
                y = jnp.dot(gm, y_s[ch], preferred_element_type=F32)
                oa_s[g, pl.ds(rr, L), :] = (y * qb[g, pl.ds(rr, L), :].astype(F32)).astype(BF16)
            return carry

        lax.fori_loop(0, NJ, loop3, 0)
        oa_copy(g).start()
        return carry

    lax.fori_loop(0, NG, g_body, 0)

    def p2(j, carry):
        r = pl.multiple_of(j * TB, TB)
        lhs = jnp.concatenate([pqn_s[g, pl.ds(r, TB), :] for g in range(NG)], axis=1)
        ob_s[j] = jnp.dot(lhs, m_s[...], preferred_element_type=F32).astype(BF16)
        ob_copy(j).start()
        return carry

    lax.fori_loop(0, NJ, p2, 0)
    for g in range(NG):
        oa_copy(g).wait()
    for j in range(NJ):
        ob_copy(j).wait()


@jax.jit
def pallas_concat_heads__ssm_conv_h3__linear_attn_block__prompt_kernel(
    A_q: jax.Array,
    A_k: jax.Array,
    A_v: jax.Array,
    A_shift_k: jax.Array,
    A_ssm_k: jax.Array,
    A_ssm_D: jax.Array,
    B_x: jax.Array,
    B_wqkv: jax.Array,
    B_wo: jax.Array,
):
    fwd, inv = _dft_mats()
    hbm = pl.BlockSpec(memory_space=pl.ANY)
    vm = pl.BlockSpec(memory_space=pltpu.VMEM)
    out = pl.pallas_call(
        _kernel,
        out_shape=jax.ShapeDtypeStruct((S, 2 * D), BF16),
        in_specs=[hbm, hbm, hbm, vm, hbm, vm, hbm, hbm, hbm, vm, vm],
        out_specs=hbm,
        scratch_shapes=[
            pltpu.VMEM((NG, S, CT), BF16),
            pltpu.VMEM((NG, S + PAD, CT), BF16),
            pltpu.VMEM((NG, S, CT), BF16),
            pltpu.VMEM((NG, CT, S), BF16),
            pltpu.VMEM((S, D), BF16),
            pltpu.VMEM((NG, D, 3 * CT), BF16),
            pltpu.VMEM((NG, CT, D), BF16),
            pltpu.VMEM((NC, 2 * L, CT), F32),
            pltpu.VMEM((NC, 2 * L, CT), F32),
            pltpu.VMEM((NC, 2 * L, CT), BF16),
            pltpu.VMEM((S, CT), BF16),
            pltpu.VMEM((NG, S, CT), BF16),
            pltpu.VMEM((D, D), BF16),
            pltpu.VMEM((8, D), F32),
            pltpu.VMEM((NG, S, CT), BF16),
            pltpu.VMEM((NJ, TB, D), BF16),
            pltpu.SemaphoreType.DMA((8, NG)),
            pltpu.SemaphoreType.DMA((NJ,)),
            pltpu.SemaphoreType.DMA((NG,)),
            pltpu.SemaphoreType.DMA((NJ,)),
        ],
        compiler_params=pltpu.CompilerParams(vmem_limit_bytes=100 * 1024 * 1024),
    )(A_q.reshape(S, D), A_k.reshape(S, D), A_v.reshape(S, D), A_shift_k, A_ssm_k,
      A_ssm_D.reshape(1, D), B_x.reshape(S, D), B_wqkv, B_wo, fwd, inv)
    return out.reshape(1, S, 2 * D)
```

```python
import numpy as np
import jax
import jax.numpy as jnp
from jax import lax
import jax.experimental.pallas as pl
import jax.experimental.pallas.tpu as pltpu

S = 2048
D = 1024
CT = 128
NG = D // CT
L = 128
NC = S // L
TB = 256
NJ = S // TB
PAD = 16
T1, T2, T3 = 512, 512, 1024
NFREE, GSPAN = 2, 0.8
DH = 32

F32 = jnp.float32
BF16 = jnp.bfloat16
U32 = jnp.uint32


def _dft_mats():
    f = np.concatenate([np.arange(0, L, 2), np.arange(1, L, 2)]).astype(np.float64)
    a = np.arange(L, dtype=np.float64)
    ang = 2.0 * np.pi * np.outer(f + 0.5, a) / (2 * L)
    fwd = np.concatenate([np.cos(ang), -np.sin(ang)], axis=0)
    inv = fwd.T / L
    return fwd.astype(BF16), inv.astype(BF16)


def _phi(t):
    return jnp.where(t > 0, t + 1.0, jnp.exp(t)) + 1e-6


def _kernel(q_hbm, k_hbm, v_hbm, shk_ref, ssm_hbm, d_ref, x_hbm, w_hbm, wo_hbm,
            f_ref, g_ref, out_hbm,
            qb, kb, vb, sb, xb, wb, wob, u_s, kf_s, y_s, pkt_s, v_s, pqn_s, m_s,
            par_s, one_s, oa_s, ob_s, in_sem, x_sem, oa_sem, ob_sem):

    def in_copies(g):
        c = pl.multiple_of(g * CT, CT)
        return [
            pltpu.make_async_copy(w_hbm.bitcast(U32).at[:, pl.ds(D + c, CT)], wb.at[g, 0], in_sem.at[0, g]),
            pltpu.make_async_copy(k_hbm.at[:, pl.ds(c, CT)], kb.at[g, pl.ds(PAD, S), :], in_sem.at[1, g]),
            pltpu.make_async_copy(v_hbm.at[:, pl.ds(c, CT)], vb.at[g], in_sem.at[2, g]),
            pltpu.make_async_copy(ssm_hbm.at[pl.ds(c, CT), :], sb.at[g], in_sem.at[3, g]),
            pltpu.make_async_copy(w_hbm.bitcast(U32).at[:, pl.ds(2 * D + c, CT)], wb.at[g, 1], in_sem.at[4, g]),
            pltpu.make_async_copy(w_hbm.bitcast(U32).at[:, pl.ds(c, CT)], wb.at[g, 2], in_sem.at[5, g]),
            pltpu.make_async_copy(wo_hbm.at[pl.ds(c, CT), :], wob.at[g], in_sem.at[6, g]),
            pltpu.make_async_copy(q_hbm.at[:, pl.ds(c, CT)], qb.at[g], in_sem.at[7, g]),
        ]

    def x_copy(j):
        r2 = pl.multiple_of(j * (TB // 2), TB // 2)
        return [pltpu.make_async_copy(x_hbm.bitcast(U32).at[pl.ds(r2, TB // 2), pl.ds(kt * CT, CT)], xb.at[kt, pl.ds(r2, TB // 2), :], x_sem.at[j])
                for kt in range(NG)]

    def oa_copy(g):
        c = pl.multiple_of(g * CT, CT)
        return pltpu.make_async_copy(oa_s.at[g], out_hbm.at[:, pl.ds(c, CT)], oa_sem.at[g])

    def ob_copy(j):
        r = pl.multiple_of(j * TB, TB)
        return pltpu.make_async_copy(ob_s.at[j], out_hbm.at[pl.ds(r, TB), pl.ds(D, D)], ob_sem.at[j])

    c0 = in_copies(0)
    c0[0].start()
    for cp in x_copy(0):
        cp.start()
    for cp in c0[1:4]:
        cp.start()
    for j in range(1, NJ):
        for cp in x_copy(j):
            cp.start()
    for cp in c0[4:]:
        cp.start()

    for g in range(NG):
        kb[g, 0:PAD, :] = jnp.zeros((PAD, CT), BF16)
    par_s[0:4, :] = shk_ref[...].astype(F32)
    one_s[...] = jnp.ones((32, CT), F32)
    par_s[4:5, :] = d_ref[...].astype(F32)

    ri = lax.broadcasted_iota(jnp.int32, (CT, CT), 0) // DH
    ci = lax.broadcasted_iota(jnp.int32, (CT, CT), 1) // DH
    bd_mask = ri == ci

    def g_body(g, carry):
        cps = in_copies(g)

        @pl.when(g + 1 < NG)
        def _():
            for cp in in_copies(g + 1):
                cp.start()

        for cp in cps[0:4]:
            cp.wait()
        c = pl.multiple_of(g * CT, CT)
        par = par_s[:, pl.ds(c, CT)]

        def ldx(j, tb, kts):
            r2 = pl.multiple_of(j * (tb // 2), tb // 2)
            return jnp.concatenate([pltpu.bitcast(xb[kt, pl.ds(r2, tb // 2), :], BF16) for kt in kts], axis=1)

        def loop1(j, z):
            @pl.when(g == 0)
            def _():
                for i in range(T1 // TB):
                    for cp in x_copy(j * (T1 // TB) + i):
                        cp.wait()
            r = pl.multiple_of(j * T1, T1)
            kk = jnp.dot(ldx(j, T1, range(NG)), pltpu.bitcast(wb[g, 0], BF16), preferred_element_type=F32)
            pk = _phi(kk)
            pkt_s[:, pl.ds(r, T1)] = pk.T.astype(BF16)
            z = z + pk.reshape(T1 // 8, 8, CT).sum(axis=0)
            ka = kb[g, pl.ds(r, T1 + PAD), :].astype(F32)
            ks = ka[PAD:PAD + T1] * par[0:1]
            for t in range(1, 4):
                ks = ks + ka[PAD - t:PAD - t + T1] * par[t:t + 1]
            kv = (ks * vb[g, pl.ds(r, T1), :].astype(F32)).astype(BF16)
            fm = f_ref[...]
            for h in range(T1 // L):
                ch = j * (T1 // L) + h
                u_s[ch] = jnp.dot(fm, kv[h * L:(h + 1) * L], preferred_element_type=F32)
                kt = sb[g, :, pl.ds(pl.multiple_of(r + h * L, L), L)]
                kf_s[ch] = lax.dot_general(fm, kt, (((1,), (1,)), ((), ())),
                                           preferred_element_type=F32)
            return z

        z = lax.fori_loop(0, S // T1, loop1, jnp.zeros((8, CT), F32))
        z = jnp.sum(z, axis=0, keepdims=True)
        zbd_t = jnp.where(bd_mask, z, 0.0).astype(BF16)
        cps[4].wait()
        cps[5].wait()
        dvec = par[4:5]

        def loop2(j, carry):
            r = pl.multiple_of(j * T2, T2)
            xh = [ldx(j, T2, range(4 * h, 4 * h + 4)) for h in range(2)]
            rounds = [jnp.dot(xh[h], pltpu.bitcast(wb[g, w, h * 256:(h + 1) * 256], BF16),
                              preferred_element_type=F32) for w in (2, 1) for h in range(2)]
            pqn_s[g, pl.ds(r, T2), :] = _phi(rounds[0] + rounds[1]).astype(BF16)
            v_s[pl.ds(r, T2), :] = (rounds[2] + rounds[3]).astype(BF16)
            one_a = one_s[0:16]
            one_b = one_s[16:32]
            rows = 16
            nsub = L * T2 // S // rows
            B = 4
            npairs = nsub * 10

            def gate(n):
                if n < NFREE:
                    return None
                pos = int((n - NFREE) * GSPAN * 4 * T2) // (npairs - NFREE)
                rd, row = pos // T2, (pos % T2) // 16 * 16
                return jnp.where(rounds[rd][row:row + 16] > 0, one_a, one_b)

            sgn = jnp.where(j < S // T2 // 2, 1.0, -1.0).astype(F32)
            npair = 0
            for sub in range(nsub):
                p = pl.multiple_of((j * nsub + sub) * rows, rows)

                def ld(ref, ch):
                    return ref[ch, pl.ds(p, rows), :], ref[ch, pl.ds(L + p, rows), :]

                prev = None
                for cb in range(NC // B):
                    acc = [None] * B
                    for jb in range(cb + 1):
                        gt = gate(npair)
                        npair += 1
                        us = [ld(u_s, jb * B + i) for i in range(B)]
                        if gt is not None:
                            us = [(a * gt, b * gt) for a, b in us]
                        for m in range((cb - jb) * B - (B - 1), (cb - jb) * B + B):
                            if m < 0:
                                continue
                            kr, ki = ld(kf_s, m)
                            if m == 0:
                                kr = kr + dvec
                            for i in range(B):
                                cc = jb * B + i + m - cb * B
                                if 0 <= cc < B:
                                    ur, ui = us[i]
                                    tr = ur * kr - ui * ki
                                    ti = ur * ki + ui * kr
                                    if acc[cc] is None:
                                        acc[cc] = (tr, ti)
                                    else:
                                        acc[cc] = (acc[cc][0] + tr, acc[cc][1] + ti)
                    for i in range(B):
                        yr, yi = acc[i]
                        if prev is not None:
                            yr, yi = yr - sgn * prev[1], yi + sgn * prev[0]
                        prev = acc[i]
                        y_s[cb * B + i, pl.ds(p, rows), :] = yr.astype(BF16)
                        y_s[cb * B + i, pl.ds(L + p, rows), :] = yi.astype(BF16)
            return carry

        lax.fori_loop(0, S // T2, loop2, 0)
        cps[6].wait()
        cps[7].wait()

        def loop3(j, kvacc):
            r = pl.multiple_of(j * T3, T3)
            kvacc = kvacc + jnp.dot(pkt_s[:, pl.ds(r, T3)], v_s[pl.ds(r, T3), :], preferred_element_type=F32)
            q4 = T3 // 4
            for i in range(4):
                rr = pl.multiple_of(r + i * q4, q4)
                pq = pqn_s[g, pl.ds(rr, q4), :]
                den = lax.dot_general(pq, zbd_t, (((1,), (1,)), ((), ())), preferred_element_type=F32) + 1e-6
                rc = pl.reciprocal(den, approx=True)
                rc = rc * (2.0 - den * rc)
                pqn_s[g, pl.ds(rr, q4), :] = (pq.astype(F32) * rc).astype(BF16)
            gm = g_ref[...]
            for h in range(T3 // L):
                ch = j * (T3 // L) + h
                rr = pl.multiple_of(ch * L, L)
                y = jnp.dot(gm, y_s[ch], preferred_element_type=F32)
                oa_s[g, pl.ds(rr, L), :] = (y * qb[g, pl.ds(rr, L), :].astype(F32)).astype(BF16)
            return kvacc

        kvacc = lax.fori_loop(0, S // T3, loop3, jnp.zeros((CT, CT), F32))
        kvm = jnp.where(bd_mask, kvacc, 0.0).astype(BF16)
        m_s[pl.ds(c, CT), :] = jnp.dot(kvm, wob[g], preferred_element_type=F32).astype(BF16)
        oa_copy(g).start()
        return carry

    lax.fori_loop(0, NG, g_body, 0)

    def p2(j, carry):
        r = pl.multiple_of(j * TB, TB)
        lhs = jnp.concatenate([pqn_s[g, pl.ds(r, TB), :] for g in range(NG)], axis=1)
        ob_s[j] = jnp.dot(lhs, m_s[...], preferred_element_type=F32).astype(BF16)
        ob_copy(j).start()
        return carry

    lax.fori_loop(0, NJ, p2, 0)
    for g in range(NG):
        oa_copy(g).wait()
    for j in range(NJ):
        ob_copy(j).wait()


@jax.jit
def pallas_concat_heads__ssm_conv_h3__linear_attn_block__prompt_kernel(
    A_q: jax.Array,
    A_k: jax.Array,
    A_v: jax.Array,
    A_shift_k: jax.Array,
    A_ssm_k: jax.Array,
    A_ssm_D: jax.Array,
    B_x: jax.Array,
    B_wqkv: jax.Array,
    B_wo: jax.Array,
):
    fwd, inv = _dft_mats()
    hbm = pl.BlockSpec(memory_space=pl.ANY)
    vm = pl.BlockSpec(memory_space=pltpu.VMEM)
    out = pl.pallas_call(
        _kernel,
        out_shape=jax.ShapeDtypeStruct((S, 2 * D), BF16),
        in_specs=[hbm, hbm, hbm, vm, hbm, vm, hbm, hbm, hbm, vm, vm],
        out_specs=hbm,
        scratch_shapes=[
            pltpu.VMEM((NG, S, CT), BF16),
            pltpu.VMEM((NG, S + PAD, CT), BF16),
            pltpu.VMEM((NG, S, CT), BF16),
            pltpu.VMEM((NG, CT, S), BF16),
            pltpu.VMEM((NG, S // 2, CT), U32),
            pltpu.VMEM((NG, 3, D // 2, CT), U32),
            pltpu.VMEM((NG, CT, D), BF16),
            pltpu.VMEM((NC, 2 * L, CT), F32),
            pltpu.VMEM((NC, 2 * L, CT), F32),
            pltpu.VMEM((NC, 2 * L, CT), BF16),
            pltpu.VMEM((CT, S), BF16),
            pltpu.VMEM((S, CT), BF16),
            pltpu.VMEM((NG, S, CT), BF16),
            pltpu.VMEM((D, D), BF16),
            pltpu.VMEM((8, D), F32),
            pltpu.VMEM((32, CT), F32),
            pltpu.VMEM((NG, S, CT), BF16),
            pltpu.VMEM((NJ, TB, D), BF16),
            pltpu.SemaphoreType.DMA((8, NG)),
            pltpu.SemaphoreType.DMA((NJ,)),
            pltpu.SemaphoreType.DMA((NG,)),
            pltpu.SemaphoreType.DMA((NJ,)),
        ],
        compiler_params=pltpu.CompilerParams(vmem_limit_bytes=100 * 1024 * 1024),
    )(A_q.reshape(S, D), A_k.reshape(S, D), A_v.reshape(S, D), A_shift_k.T, A_ssm_k,
      A_ssm_D.reshape(1, D), B_x.reshape(S, D), B_wqkv, B_wo, fwd, inv)
    return out.reshape(1, S, 2 * D)
```

```python
import numpy as np
import jax
import jax.numpy as jnp
from jax import lax
import jax.experimental.pallas as pl
import jax.experimental.pallas.tpu as pltpu

S = 2048
D = 1024
CT = 128
NG = D // CT
L = 128
NC = S // L
TB = 512
NJ = S // TB
PAD = 16
T1, T2, T3 = 512, 1024, 1024
BLK = 2
NFREE, GSPAN = 4, 0.92
DH = 32

F32 = jnp.float32
BF16 = jnp.bfloat16
U32 = jnp.uint32


def _dft_mats():
    f = np.concatenate([np.arange(0, L, 2), np.arange(1, L, 2)]).astype(np.float64)
    a = np.arange(L, dtype=np.float64)
    ang = 2.0 * np.pi * np.outer(f + 0.5, a) / (2 * L)
    fwd = np.concatenate([np.cos(ang), -np.sin(ang)], axis=0)
    inv = fwd.T / L
    return fwd.astype(BF16), inv.astype(BF16)


def _phi(t):
    return jnp.where(t > 0, t + 1.0, jnp.exp(t)) + 1e-6


def _kernel(q_hbm, k_hbm, v_hbm, shk_ref, ssm_hbm, d_ref, x_hbm, w_hbm, wo_hbm,
            f_ref, g_ref, out_hbm,
            qb, kb, vb, sb, xb, wb, wob, u_s, kf_s, kp_s, y_s, pkt_s, v_s, pq_s, pqn_s, m_s, kvm_s,
            par_s, one_s, oa_s, ob_s, in_sem, x_sem, oa_sem, ob_sem):

    def in_copies(g, sel=range(8)):
        c = pl.multiple_of(g * CT, CT)
        args = [
            (w_hbm.bitcast(U32).at[:, pl.ds(D + c, CT)], wb.at[g, 0], in_sem.at[0, g]),
            (k_hbm.at[:, pl.ds(c, CT)], kb.at[g, pl.ds(PAD, S), :], in_sem.at[1, g]),
            (v_hbm.at[:, pl.ds(c, CT)], vb.at[g], in_sem.at[2, g]),
            (ssm_hbm.at[pl.ds(c, CT), :], sb.at[g], in_sem.at[3, g]),
            (w_hbm.bitcast(U32).at[:, pl.ds(2 * D + c, CT)], wb.at[g, 1], in_sem.at[4, g]),
            (w_hbm.bitcast(U32).at[:, pl.ds(c, CT)], wb.at[g, 2], in_sem.at[5, g]),
            (wo_hbm.at[pl.ds(c, CT), :], wob.at[g], in_sem.at[6, g]),
            (q_hbm.at[:, pl.ds(c, CT)], qb.at[g], in_sem.at[7, g]),
        ]
        return [pltpu.make_async_copy(*args[i]) for i in sel]

    def x_copy(j):
        r2 = pl.multiple_of(j * (T1 // 2), T1 // 2)
        return [pltpu.make_async_copy(x_hbm.bitcast(U32).at[pl.ds(r2, T1 // 2), pl.ds(kt * CT, CT)], xb.at[kt, pl.ds(r2, T1 // 2), :], x_sem.at[j])
                for kt in range(NG)]

    def oa_copy(g):
        c = pl.multiple_of(g * CT, CT)
        return pltpu.make_async_copy(oa_s.at[g], out_hbm.at[:, pl.ds(c, CT)], oa_sem.at[g])

    def ob_copy(j):
        r = pl.multiple_of(j * TB, TB)
        return pltpu.make_async_copy(ob_s.at[j], out_hbm.at[pl.ds(r, TB), pl.ds(D, D)], ob_sem.at[j])

    def first_copies(j):
        r = pl.multiple_of(j * T1, T1)
        cps = [
            pltpu.make_async_copy(k_hbm.at[pl.ds(r, T1), 0:CT], kb.at[0, pl.ds(PAD + r, T1), :], x_sem.at[j]),
            pltpu.make_async_copy(v_hbm.at[pl.ds(r, T1), 0:CT], vb.at[0, pl.ds(r, T1), :], x_sem.at[j]),
            pltpu.make_async_copy(ssm_hbm.at[0:CT, pl.ds(r, T1)], sb.at[0, :, pl.ds(r, T1)], x_sem.at[j]),
        ]
        return x_copy(j) + cps

    in_copies(0, [0])[0].start()
    for cp in first_copies(0) + first_copies(1):
        cp.start()

    for g in range(NG):
        kb[g, 0:PAD, :] = jnp.zeros((PAD, CT), BF16)
    par_s[0:4, :] = shk_ref[...].astype(F32)
    one_s[...] = jnp.ones((32, CT), F32)
    par_s[4:5, :] = d_ref[...].astype(F32).reshape(1, D)

    ri = lax.broadcasted_iota(jnp.int32, (CT, CT), 0) // DH
    ci = lax.broadcasted_iota(jnp.int32, (CT, CT), 1) // DH
    bd_mask = ri == ci

    def g_body(g, carry):

        @pl.when(g > 0)
        def _():
            for cp in in_copies(g, range(1, 4)):
                cp.wait()

            @pl.when(g + 1 < NG)
            def _():
                for cp in in_copies(g + 1):
                    cp.start()

        in_copies(g, [0])[0].wait()
        c = pl.multiple_of(g * CT, CT)
        par = par_s[:, pl.ds(c, CT)]

        def ldx(j, tb, kts):
            r2 = pl.multiple_of(j * (tb // 2), tb // 2)
            return jnp.concatenate([pltpu.bitcast(xb[kt, pl.ds(r2, tb // 2), :], BF16) for kt in kts], axis=1)

        def loop1(j, z):
            @pl.when(g == 0)
            def _():
                @pl.when(j + 2 < S // T1)
                def _():
                    for cp in first_copies(j + 2):
                        cp.start()

                @pl.when(j + 2 == S // T1)
                def _():
                    for cp in in_copies(0, range(4, 8)) + in_copies(1):
                        cp.start()

                for cp in first_copies(j):
                    cp.wait()
            r = pl.multiple_of(j * T1, T1)
            kk = jnp.dot(ldx(j, T1, range(NG)), pltpu.bitcast(wb[g, 0], BF16), preferred_element_type=F32)
            pk = _phi(kk)
            pkt_s[:, pl.ds(r, T1)] = pk.T.astype(BF16)
            z = z + pk.reshape(T1 // 8, 8, CT).sum(axis=0)
            ka = kb[g, pl.ds(r, T1 + PAD), :].astype(F32)
            ks = ka[PAD:PAD + T1] * par[0:1]
            for t in range(1, 4):
                ks = ks + ka[PAD - t:PAD - t + T1] * par[t:t + 1]
            kv = (ks * vb[g, pl.ds(r, T1), :].astype(F32)).astype(BF16)
            fm = f_ref[...]
            kp = kp_s[...]
            for h in range(T1 // L):
                ch = j * (T1 // L) + h
                uu = jnp.dot(fm, kv[h * L:(h + 1) * L], preferred_element_type=F32)
                u_s[ch, 0:2 * L] = uu
                u_s[ch, 2 * L:3 * L] = uu[0:L] + uu[L:2 * L]
                kt = sb[g, :, pl.ds(pl.multiple_of(r + h * L, L), L)]
                kf = lax.dot_general(fm, kt, (((1,), (1,)), ((), ())), preferred_element_type=F32)
                H = L // 2
                cr = jnp.concatenate([kf[0:H] - kp[L:L + H], kf[H:L] + kp[L + H:2 * L]], axis=0)
                ci = jnp.concatenate([kf[L:L + H] + kp[0:H], kf[L + H:2 * L] - kp[H:L]], axis=0)
                if h == 0:
                    cr = cr + jnp.where(j == 0, par[4:5], 0.0)
                kp = kf
                kf_s[ch, 0:L] = cr
                kf_s[ch, L:2 * L] = ci - cr
                kf_s[ch, 2 * L:3 * L] = ci + cr
            kp_s[...] = kp
            return z

        kp_s[...] = jnp.zeros((2 * L, CT), F32)
        z = lax.fori_loop(0, S // T1, loop1, jnp.zeros((8, CT), F32))
        z = jnp.sum(z, axis=0, keepdims=True)
        zbd_t = jnp.where(bd_mask, z, 0.0).astype(BF16)
        in_copies(g, [4])[0].wait()
        in_copies(g, [5])[0].wait()

        def loop2(j, carry):
            r = pl.multiple_of(j * T2, T2)
            xh = [ldx(j, T2, range(4 * h, 4 * h + 4)) for h in range(2)]
            rounds = [jnp.dot(xh[h], pltpu.bitcast(wb[g, w, h * 256:(h + 1) * 256], BF16),
                              preferred_element_type=F32) for w in (2, 1) for h in range(2)]
            pq_s[pl.ds(r, T2), :] = _phi(rounds[0] + rounds[1]).astype(BF16)
            v_s[pl.ds(r, T2), :] = (rounds[2] + rounds[3]).astype(BF16)
            one_a = one_s[0:16]
            one_b = one_s[16:32]
            rows = 16
            nsub = L * T2 // S // rows
            B = BLK
            npairs = nsub * (NC // B) * (NC // B + 1) // 2

            def gate(n):
                if n < NFREE:
                    return None
                pos = int((n - NFREE) * GSPAN * 4 * T2) // (npairs - NFREE)
                rd, row = pos // T2, (pos % T2) // 16 * 16
                return jnp.where(rounds[rd][row:row + 16] > 0, one_a, one_b)

            npair = 0
            for sub in range(nsub):
                p = pl.multiple_of((j * nsub + sub) * rows, rows)

                def ld(ref, ch):
                    return [ref[ch, pl.ds(i * L + p, rows), :] for i in range(3)]

                for cb in range(NC // B):
                    acc = [None] * B
                    for jb in range(cb + 1):
                        gt = gate(npair)
                        npair += 1
                        us = [ld(u_s, jb * B + i) for i in range(B)]
                        if gt is not None:
                            us = [[t * gt for t in u3] for u3 in us]
                        for m in range((cb - jb) * B - (B - 1), (cb - jb) * B + B):
                            if m < 0:
                                continue
                            kc, kd, ke = ld(kf_s, m)
                            for i in range(B):
                                cc = jb * B + i + m - cb * B
                                if 0 <= cc < B:
                                    ua, ub, uc = us[i]
                                    t3 = [uc * kc, ua * kd, ub * ke]
                                    if acc[cc] is None:
                                        acc[cc] = t3
                                    else:
                                        acc[cc] = [x + y for x, y in zip(acc[cc], t3)]
                    for i in range(B):
                        yr, yi = acc[i][0] - acc[i][2], acc[i][0] + acc[i][1]
                        y_s[cb * B + i, pl.ds(p, rows), :] = yr.astype(BF16)
                        y_s[cb * B + i, pl.ds(L + p, rows), :] = yi.astype(BF16)
            return carry

        lax.fori_loop(0, S // T2, loop2, 0)
        in_copies(g, [6])[0].wait()
        in_copies(g, [7])[0].wait()

        def loop3(j, kvacc):
            r = pl.multiple_of(j * T3, T3)
            kvacc = kvacc + jnp.dot(pkt_s[:, pl.ds(r, T3)], v_s[pl.ds(r, T3), :], preferred_element_type=F32)
            q4 = T3 // 4
            for i in range(4):
                rr = pl.multiple_of(r + i * q4, q4)
                pq = pq_s[pl.ds(rr, q4), :]
                den = lax.dot_general(pq, zbd_t, (((1,), (1,)), ((), ())), preferred_element_type=F32) + 1e-6
                rc = pl.reciprocal(den, approx=True)
                rc = rc * (2.0 - den * rc)
                pqn_s[g, pl.ds(rr, q4), :] = (pq.astype(F32) * rc).astype(BF16)
            gm = g_ref[...]
            for h in range(T3 // L):
                ch = j * (T3 // L) + h
                rr = pl.multiple_of(ch * L, L)
                y = jnp.dot(gm, y_s[ch], preferred_element_type=F32)
                oa_s[g, pl.ds(rr, L), :] = (y * qb[g, pl.ds(rr, L), :].astype(F32)).astype(BF16)
            return kvacc

        kvacc = lax.fori_loop(0, S // T3, loop3, jnp.zeros((CT, CT), F32))
        kvm = jnp.where(bd_mask, kvacc, 0.0).astype(BF16)
        kvm_s[g] = kvm
        oa_copy(g).start()
        return carry

    lax.fori_loop(0, NG, g_body, 0)

    for g in range(NG):
        m_s[g * CT:(g + 1) * CT, :] = jnp.dot(kvm_s[g], wob[g], preferred_element_type=F32).astype(BF16)

    def p2(j, carry):
        r = pl.multiple_of(j * TB, TB)
        lhs = jnp.concatenate([pqn_s[g, pl.ds(r, TB), :] for g in range(NG)], axis=1)
        ob_s[j] = jnp.dot(lhs, m_s[...], preferred_element_type=F32).astype(BF16)
        ob_copy(j).start()
        return carry

    lax.fori_loop(0, NJ, p2, 0)
    for g in range(NG):
        oa_copy(g).wait()
    for j in range(NJ):
        ob_copy(j).wait()


@jax.jit
def pallas_concat_heads__ssm_conv_h3__linear_attn_block__prompt_kernel(
    A_q: jax.Array,
    A_k: jax.Array,
    A_v: jax.Array,
    A_shift_k: jax.Array,
    A_ssm_k: jax.Array,
    A_ssm_D: jax.Array,
    B_x: jax.Array,
    B_wqkv: jax.Array,
    B_wo: jax.Array,
):
    fwd, inv = _dft_mats()
    hbm = pl.BlockSpec(memory_space=pl.ANY)
    vm = pl.BlockSpec(memory_space=pltpu.VMEM)
    out = pl.pallas_call(
        _kernel,
        out_shape=jax.ShapeDtypeStruct((S, 2 * D), BF16),
        in_specs=[hbm, hbm, hbm, vm, hbm, vm, hbm, hbm, hbm, vm, vm],
        out_specs=hbm,
        scratch_shapes=[
            pltpu.VMEM((NG, S, CT), BF16),
            pltpu.VMEM((NG, S + PAD, CT), BF16),
            pltpu.VMEM((NG, S, CT), BF16),
            pltpu.VMEM((NG, CT, S), BF16),
            pltpu.VMEM((NG, S // 2, CT), U32),
            pltpu.VMEM((NG, 3, D // 2, CT), U32),
            pltpu.VMEM((NG, CT, D), BF16),
            pltpu.VMEM((NC, 3 * L, CT), F32),
            pltpu.VMEM((NC, 3 * L, CT), F32),
            pltpu.VMEM((2 * L, CT), F32),
            pltpu.VMEM((NC, 2 * L, CT), BF16),
            pltpu.VMEM((CT, S), BF16),
            pltpu.VMEM((S, CT), BF16),
            pltpu.VMEM((S, CT), BF16),
            pltpu.VMEM((NG, S, CT), BF16),
            pltpu.VMEM((D, D), BF16),
            pltpu.VMEM((NG, CT, CT), BF16),
            pltpu.VMEM((8, D), F32),
            pltpu.VMEM((32, CT), F32),
            pltpu.VMEM((NG, S, CT), BF16),
            pltpu.VMEM((NJ, TB, D), BF16),
            pltpu.SemaphoreType.DMA((8, NG)),
            pltpu.SemaphoreType.DMA((S // T1,)),
            pltpu.SemaphoreType.DMA((NG,)),
            pltpu.SemaphoreType.DMA((NJ,)),
        ],
        compiler_params=pltpu.CompilerParams(vmem_limit_bytes=100 * 1024 * 1024),
    )(A_q.reshape(S, D), A_k.reshape(S, D), A_v.reshape(S, D), A_shift_k.T, A_ssm_k,
      A_ssm_D, B_x.reshape(S, D), B_wqkv, B_wo, fwd, inv)
    return out.reshape(1, S, 2 * D)
```
